```python
import jax
import jax.numpy as jnp

def _softmax(x, axis=-1):
    return jax.nn.softmax(x, axis=axis)
def _gelu(x):
    return jax.nn.gelu(x, approximate=True)
def _silu(x):
    return jax.nn.silu(x)
def _sigmoid(x):
    return jax.nn.sigmoid(x)
def _layernorm(x, axis=-1, eps=1e-5):
    m = jnp.mean(x, axis=axis, keepdims=True)
    v = jnp.var(x, axis=axis, keepdims=True)
    return (x - m) / jnp.sqrt(v + eps)
def _scatter_add(tgt, idx, src, axis=0):
    return tgt.at[idx].add(src)
def _segment_sum(src, seg, n):
    return jax.ops.segment_sum(src, seg, n)
class _Rng:
    def __init__(self, key):
        self._k = key
    def _next(self):
        self._k, sub = jax.random.split(self._k)
        return sub
    def normal(self, shape):
        return jax.random.normal(self._next(), shape, dtype=jnp.bfloat16)
    def randint(self, lo, hi, shape):
        return jax.random.randint(self._next(), shape, lo, hi, dtype=jnp.int32)
    def uniform(self, shape, lo=0.0, hi=1.0):
        return jax.random.uniform(self._next(), shape, jnp.bfloat16, lo, hi)
    def permutation(self, n):
        return jax.random.permutation(self._next(), n)


kernel_name = 'gated_mix__mha_block_cached__moe_arch_mod__decode'

def setup_inputs():
    _rng = _Rng(jax.random.key(int.from_bytes(__import__("os").urandom(4), "little")))
    _w = (lambda a: (lambda t: t.astype(jnp.bfloat16) if jnp.issubdtype(t.dtype, jnp.floating) else t)(jnp.asarray(a)))
    def _A_setup():
        B, Sq, D = 4, 1, 1024
        H, Sk, Dh = 32, 8192, 128
        return {
            "x": _w((lambda *s: _rng.normal(s) * 0.05)(B, Sq, D)),
            "k_cache": _w((lambda *s: _rng.normal(s) * 0.05)(B, H, Sk, Dh)),
            "v_cache": _w((lambda *s: _rng.normal(s) * 0.05)(B, H, Sk, Dh)),
            "wq": _w((lambda *s: _rng.normal(s) * 0.05)(D, H * Dh) * (D ** -0.5)),
            "wo": _w((lambda *s: _rng.normal(s) * 0.05)(H * Dh, D) * ((H * Dh) ** -0.5)),
        }
    _A_in = _A_setup()

    def _B_setup():
        B, S, D, F, C = 4, 1, 1024, 3584, 1
        return {
            "x": _w((lambda *s: _rng.normal(s) * 0.05)(B, S, D)),
            "w_r": _w((lambda *s: _rng.normal(s) * 0.05)(D)),
            "w_gate": _w((lambda *s: _rng.normal(s) * 0.05)(D, F)),
            "w_up": _w((lambda *s: _rng.normal(s) * 0.05)(D, F)),
            "w_down": _w((lambda *s: _rng.normal(s) * 0.05)(F, D)),
        }
    _B_in = _B_setup()

    return {
        "A_x": _A_in["x"],
        "A_k_cache": _A_in["k_cache"],
        "A_v_cache": _A_in["v_cache"],
        "A_wq": _A_in["wq"],
        "A_wo": _A_in["wo"],
        "B_x": _B_in["x"],
        "B_w_r": _B_in["w_r"],
        "B_w_gate": _B_in["w_gate"],
        "B_w_up": _B_in["w_up"],
        "B_w_down": _B_in["w_down"],
        "gate_w": _w((lambda *s: _rng.normal(s) * 0.05)(1024)),
    }

def reference(A_x, A_k_cache, A_v_cache, A_wq, A_wo, B_x, B_w_r, B_w_gate, B_w_up, B_w_down, gate_w):
    def _A_ref(x, k_cache, v_cache, wq, wo):
        B, Sq, D = x.shape
        H, Dh = 32, 128
        q = (lambda x, *d: x.transpose(*d))((x @ wq).reshape(B, Sq, H, Dh), 0, 2, 1, 3)
        scores = jnp.einsum("bhqd,bhkd->bhqk", q, k_cache) * (Dh ** -0.5)
        p = _softmax(scores, axis=-1)
        o = jnp.einsum("bhqk,bhkd->bhqd", p, v_cache)
        return (lambda x, *d: x.transpose(*d))(o, 0, 2, 1, 3).reshape(B, Sq, H * Dh) @ wo

    def _B_ref(x, w_r, w_gate, w_up, w_down):
        B, S, D = x.shape
        C = 1
        r = x @ w_r
        idx = jnp.argsort(-r, axis=-1)[:, :C]
        idx_e = jnp.repeat(idx.reshape(B, C, 1), D, axis=2)
        x_sel = jnp.take_along_axis(x, idx_e, axis=1)
        g = _silu(x_sel @ w_gate)
        u = x_sel @ w_up
        y = (g * u) @ w_down
        r_sel = _sigmoid(jnp.take_along_axis(r, idx, axis=1))
        y = y * r_sel.reshape(B, C, 1)
        b_off = (jnp.arange(B) * S).reshape(B, 1)
        flat_idx = (idx + b_off).reshape(B * C)
        zero = (x * 0.0).reshape(B * S, D)
        upd = _scatter_add(zero, flat_idx, y.reshape(B * C, D), axis=0)
        return x + upd.reshape(B, S, D)

    x = A_x
    g = _sigmoid((x * gate_w).sum(-1, keepdims=True))
    a = _A_ref(x, A_k_cache, A_v_cache, A_wq, A_wo)
    b = _B_ref(x, B_w_r, B_w_gate, B_w_up, B_w_down)
    return g * a + (1 - g) * b
```

```python
import jax
import jax.numpy as jnp
import jax.experimental.pallas as pl
import jax.experimental.pallas.tpu as pltpu

B, D, H, S, DH, F = 4, 1024, 32, 8192, 128, 3584
NBH = B * H
CH = 2048
NCH = S // CH
NU = NBH * NCH
NSLOT = 4
R = 128
NP = CH // R
T_WO, T_WG, T_WU, T_WD, T_H, T_Y = 1, 8, 12, 16, 24, 28


def _kernel(x_hbm, wr_hbm, gw_hbm, k_hbm, v_hbm, wq_hbm, wo_hbm, wg_hbm, wu_hbm, wd_hbm,
            o_ref,
            x_v, wr_v, gw_v, wq_v, wo_v, wg_v, wu_v, wd_v, kbuf, vbuf,
            q_scr, o_scr, a_scr, h_scr, b_scr, ksem, vsem, wsem):

    def start_unit(u):
        i = u // NCH
        c = u % NCH
        slot = u % NSLOT
        h = i // B
        b = i % B
        for j in range(NP):
            rows = pl.ds(pl.multiple_of(c * CH + j * R, R), R)
            for prio, (hbm, buf, sem) in enumerate(((k_hbm, kbuf, ksem), (v_hbm, vbuf, vsem))):
                pltpu.make_async_copy(hbm.at[b, h, rows], buf.at[slot, pl.ds(j * R, R)],
                                      sem.at[slot]).start(priority=prio)

    def wait_all(buf, sem):
        pltpu.make_async_copy(buf, buf, sem).wait()

    def start_matrix(hbm, vm, sem, cols):
        rows, width = hbm.shape
        half = rows // 2

        def go(r, carry):
            for c in range(width // cols):
                for prio in range(2):
                    rs = pl.ds(pl.multiple_of(prio * half + r * 16, 16), 16)
                    cs = pl.ds(c * cols, cols)
                    pltpu.make_async_copy(hbm.at[rs, cs], vm.at[rs, cs], sem).start(priority=prio)
            return carry

        jax.lax.fori_loop(0, half // 16, go, 0)

    cp_x = pltpu.make_async_copy(x_hbm, x_v, wsem.at[5])
    cp_wr = pltpu.make_async_copy(wr_hbm, wr_v, wsem.at[6])
    cp_gw = pltpu.make_async_copy(gw_hbm, gw_v, wsem.at[7])
    start_matrix(wq_hbm, wq_v, wsem.at[0], 1024)
    cp_x.start()
    cp_wr.start()
    cp_gw.start()
    for u in range(NSLOT):
        start_unit(u)

    cp_x.wait()
    xf4 = x_v[...].astype(jnp.float32)
    xf = jnp.concatenate([xf4, xf4], axis=0)
    x8 = xf.astype(jnp.bfloat16)
    wait_all(wq_v, wsem.at[0])
    q = jnp.dot(x8, wq_v[...], preferred_element_type=jnp.float32)
    q = q.astype(jnp.bfloat16).astype(jnp.float32)
    for h in range(H):
        q_scr[h] = q[:, h * DH:(h + 1) * DH]
    a_scr[...] = jnp.zeros_like(a_scr)
    o_scr[...] = jnp.zeros_like(o_scr)

    scale = DH ** -0.5

    def body(i, carry):
        h = i // B
        b = i % B
        qb = jnp.broadcast_to(q_scr[h, pl.ds(b, 1), :], (8, DH)).astype(jnp.bfloat16)
        m = l = acc = None
        for c in range(NCH):
            u = i * NCH + c
            slot = u % NSLOT
            wait_all(kbuf.at[slot], ksem.at[slot])
            s = jax.lax.dot_general(qb, kbuf[slot], (((1,), (1,)), ((), ())),
                                    preferred_element_type=jnp.float32) * scale
            mc = jnp.max(s, axis=-1, keepdims=True)
            m_old = m
            m = mc if c == 0 else jnp.maximum(m_old, mc)
            ms = jnp.where(m == -jnp.inf, 0.0, m)
            p = jnp.exp(s - ms)
            lc = jnp.sum(p, axis=-1, keepdims=True)
            wait_all(vbuf.at[slot], vsem.at[slot])
            pv = jnp.dot(p.astype(jnp.bfloat16), vbuf[slot], preferred_element_type=jnp.float32)
            if c == 0:
                l, acc = lc, pv
            else:
                alpha = jnp.exp(m_old - ms)
                l = l * alpha + lc
                acc = acc * alpha + pv

            @pl.when(u + NSLOT < NU)
            def _():
                start_unit(u + NSLOT)

        o_scr[pl.ds(b, 1), :] = (acc / l)[0:1]

        @pl.when(i == T_WO)
        def _():
            start_matrix(wo_hbm, wo_v, wsem.at[1], 1024)

        @pl.when(i == T_WG)
        def _():
            start_matrix(wg_hbm, wg_v, wsem.at[2], 896)

        @pl.when(i == T_WU)
        def _():
            start_matrix(wu_hbm, wu_v, wsem.at[3], 896)

        @pl.when(i == T_WD)
        def _():
            start_matrix(wd_hbm, wd_v, wsem.at[4], 1024)

        @pl.when(i == B - 1)
        def _():
            wait_all(wo_v, wsem.at[1])

        @pl.when(b == B - 1)
        def _():
            a_scr[...] += jnp.dot(o_scr[...].astype(jnp.bfloat16),
                                  wo_v[pl.ds(pl.multiple_of(h * DH, DH), DH), :],
                                  preferred_element_type=jnp.float32)

        @pl.when(i == T_H)
        def _():
            wait_all(wg_v, wsem.at[2])
            wait_all(wu_v, wsem.at[3])
            g = jnp.dot(x8, wg_v[...], preferred_element_type=jnp.float32)
            up = jnp.dot(x8, wu_v[...], preferred_element_type=jnp.float32)
            h_scr[...] = g * jax.nn.sigmoid(g) * up

        @pl.when(i == T_Y)
        def _():
            wait_all(wd_v, wsem.at[4])
            cp_wr.wait()
            cp_gw.wait()
            y = jnp.dot(h_scr[...].astype(jnp.bfloat16), wd_v[...], preferred_element_type=jnp.float32)
            wr = wr_v[...].astype(jnp.float32)
            gw = gw_v[...].astype(jnp.float32)
            r = jnp.zeros((8, 128), jnp.float32)
            gs = jnp.zeros((8, 128), jnp.float32)
            for j in range(D // 128):
                xj = xf[:, j * 128:(j + 1) * 128]
                r = r + xj * wr[j:j + 1, :]
                gs = gs + xj * gw[j:j + 1, :]
            r = jnp.sum(r, axis=-1, keepdims=True)
            gg = jax.nn.sigmoid(jnp.sum(gs, axis=-1, keepdims=True))
            bb = xf + (xf * 0.0 + y * jax.nn.sigmoid(r))
            b_scr[0] = (1.0 - gg) * bb
            b_scr[1] = jnp.broadcast_to(gg, (8, D))

        return carry

    jax.lax.fori_loop(0, NBH, body, 0)
    out = b_scr[1] * a_scr[...] + b_scr[0]
    o_ref[...] = out[0:B].astype(o_ref.dtype)


@jax.jit
def pallas_gated_mix__mha_block_cached__moe_arch_mod__decode_kernel(
    A_x: jax.Array,
    A_k_cache: jax.Array,
    A_v_cache: jax.Array,
    A_wq: jax.Array,
    A_wo: jax.Array,
    B_x: jax.Array,
    B_w_r: jax.Array,
    B_w_gate: jax.Array,
    B_w_up: jax.Array,
    B_w_down: jax.Array,
    gate_w: jax.Array,
):
    del B_x
    hbm = pl.BlockSpec(memory_space=pltpu.HBM)
    out = pl.pallas_call(
        _kernel,
        in_specs=[hbm] * 10,
        out_specs=pl.BlockSpec(memory_space=pltpu.VMEM),
        out_shape=jax.ShapeDtypeStruct((B, D), jnp.bfloat16),
        scratch_shapes=[
            pltpu.VMEM((B, D), jnp.bfloat16),
            pltpu.VMEM((D // 128, 128), jnp.bfloat16),
            pltpu.VMEM((D // 128, 128), jnp.bfloat16),
            pltpu.VMEM((D, H * DH), jnp.bfloat16),
            pltpu.VMEM((H * DH, D), jnp.bfloat16),
            pltpu.VMEM((D, F), jnp.bfloat16),
            pltpu.VMEM((D, F), jnp.bfloat16),
            pltpu.VMEM((F, D), jnp.bfloat16),
            pltpu.VMEM((NSLOT, CH, DH), jnp.bfloat16),
            pltpu.VMEM((NSLOT, CH, DH), jnp.bfloat16),
            pltpu.VMEM((H, 8, DH), jnp.float32),
            pltpu.VMEM((8, DH), jnp.float32),
            pltpu.VMEM((8, D), jnp.float32),
            pltpu.VMEM((8, F), jnp.float32),
            pltpu.VMEM((2, 8, D), jnp.float32),
            pltpu.SemaphoreType.DMA((NSLOT,)),
            pltpu.SemaphoreType.DMA((NSLOT,)),
            pltpu.SemaphoreType.DMA((8,)),
        ],
        compiler_params=pltpu.CompilerParams(
            vmem_limit_bytes=64 * 1024 * 1024,
            disable_bounds_checks=True,
        ),
    )(A_x.reshape(B, D), B_w_r.reshape(D // 128, 128), gate_w.reshape(D // 128, 128),
      A_k_cache, A_v_cache, A_wq, A_wo, B_w_gate, B_w_up, B_w_down)
    return out.reshape(B, 1, D)
```

```python
import jax
import jax.numpy as jnp
import jax.experimental.pallas as pl
import jax.experimental.pallas.tpu as pltpu

B, D, H, S, DH, F = 4, 1024, 32, 8192, 128, 3584
PIECES = (192, 64) * 2
CH = sum(PIECES)
NCH = S // CH
NU = H * NCH
NSLOT = 4
WS = 8
T_WO, T_WG, T_WU, T_WD, T_H, T_Y = 0, 2, 3, 4, 6, 7


def _kernel(x_hbm, wr_hbm, gw_hbm, k_hbm, v_hbm, wq_hbm, wo_hbm, wg_hbm, wu_hbm, wd_hbm,
            o_ref,
            x_v, wr_v, gw_v, wq_v, wo_v, wg_v, wu_v, wd_v, kbuf, vbuf,
            q_scr, a_scr, h_scr, b_scr, ksem, vsem, wsem):

    def start_unit(u):
        h = u // NCH
        c = u % NCH
        slot = u % NSLOT
        off = 0
        for rows in PIECES:
            src = pl.ds(pl.multiple_of(c * CH + off, 16), rows)
            dst = pl.ds(off, rows)
            for b in range(B):
                for prio, (hbm, buf, sem) in enumerate(((k_hbm, kbuf, ksem), (v_hbm, vbuf, vsem))):
                    pltpu.make_async_copy(hbm.at[b, h, src], buf.at[slot, b, dst],
                                          sem.at[slot]).start(priority=prio)
            off += rows

    def wait_all(buf, sem):
        pltpu.make_async_copy(buf, buf, sem).wait()

    def start_matrix(hbm, vm, sem, cols):
        rows, width = hbm.shape
        part = rows // WS

        def go(r, carry):
            for c in range(width // cols):
                for p in range(WS):
                    rs = pl.ds(pl.multiple_of(p * part + r * 16, 16), 16)
                    cs = pl.ds(c * cols, cols)
                    pltpu.make_async_copy(hbm.at[rs, cs], vm.at[rs, cs], sem).start(priority=p % 2)
            return carry

        jax.lax.fori_loop(0, part // 16, go, 0)

    cp_x = pltpu.make_async_copy(x_hbm, x_v, wsem.at[5])
    cp_wr = pltpu.make_async_copy(wr_hbm, wr_v, wsem.at[6])
    cp_gw = pltpu.make_async_copy(gw_hbm, gw_v, wsem.at[7])
    start_matrix(wq_hbm, wq_v, wsem.at[0], 1024)
    cp_x.start()
    cp_wr.start()
    cp_gw.start()

    def prime(u, carry):
        start_unit(u)
        return carry

    jax.lax.fori_loop(0, NSLOT, prime, 0)

    cp_x.wait()
    xf4 = x_v[...].astype(jnp.float32)
    xf = jnp.concatenate([xf4, xf4], axis=0)
    x8 = xf.astype(jnp.bfloat16)
    wait_all(wq_v, wsem.at[0])
    q = jnp.dot(x8, wq_v[...], preferred_element_type=jnp.float32)
    q = q.astype(jnp.bfloat16).astype(jnp.float32)
    for h in range(H):
        q_scr[h] = q[:, h * DH:(h + 1) * DH]
    a_scr[...] = jnp.zeros_like(a_scr)

    scale = DH ** -0.5
    batch_s = jax.lax.broadcasted_iota(jnp.int32, (8, CH), 0) % B
    batch_o = jax.lax.broadcasted_iota(jnp.int32, (8, DH), 0) % B

    def body(h, carry):
        qh = q_scr[h].astype(jnp.bfloat16)
        m = l = acc = None
        for c in range(NCH):
            u = h * NCH + c
            slot = u % NSLOT
            wait_all(kbuf.at[slot], ksem.at[slot])
            s = None
            for b in range(B):
                sb = jax.lax.dot_general(qh, kbuf[slot, b], (((1,), (1,)), ((), ())),
                                         preferred_element_type=jnp.float32)
                s = sb if b == 0 else jnp.where(batch_s == b, sb, s)
            s = s * scale
            mc = jnp.max(s, axis=-1, keepdims=True)
            m_old = m
            m = mc if c == 0 else jnp.maximum(m_old, mc)
            ms = jnp.where(m == -jnp.inf, 0.0, m)
            p = jnp.exp(s - ms)
            lc = jnp.sum(p, axis=-1, keepdims=True)
            wait_all(vbuf.at[slot], vsem.at[slot])
            pb = p.astype(jnp.bfloat16)
            pv = None
            for b in range(B):
                ob = jnp.dot(pb, vbuf[slot, b], preferred_element_type=jnp.float32)
                pv = ob if b == 0 else jnp.where(batch_o == b, ob, pv)
            if c == 0:
                l, acc = lc, pv
            else:
                alpha = jnp.exp(m_old - ms)
                l = l * alpha + lc
                acc = acc * alpha + pv

            @pl.when(u + NSLOT < NU)
            def _():
                start_unit(u + NSLOT)

            if c == 0:
                @pl.when(h == T_WO)
                def _():
                    start_matrix(wo_hbm, wo_v, wsem.at[1], 1024)

                @pl.when(h == T_WG)
                def _():
                    start_matrix(wg_hbm, wg_v, wsem.at[2], 896)

                @pl.when(h == T_WU)
                def _():
                    start_matrix(wu_hbm, wu_v, wsem.at[3], 896)

                @pl.when(h == T_WD)
                def _():
                    start_matrix(wd_hbm, wd_v, wsem.at[4], 1024)

        @pl.when(h == T_WO)
        def _():
            wait_all(wo_v, wsem.at[1])

        o = (acc / l).astype(jnp.bfloat16)
        a_scr[...] += jnp.dot(o, wo_v[pl.ds(pl.multiple_of(h * DH, DH), DH), :],
                              preferred_element_type=jnp.float32)

        @pl.when(h == T_H)
        def _():
            wait_all(wg_v, wsem.at[2])
            wait_all(wu_v, wsem.at[3])
            g = jnp.dot(x8, wg_v[...], preferred_element_type=jnp.float32)
            up = jnp.dot(x8, wu_v[...], preferred_element_type=jnp.float32)
            h_scr[...] = g * jax.nn.sigmoid(g) * up

        @pl.when(h == T_Y)
        def _():
            wait_all(wd_v, wsem.at[4])
            cp_wr.wait()
            cp_gw.wait()
            y = jnp.dot(h_scr[...].astype(jnp.bfloat16), wd_v[...], preferred_element_type=jnp.float32)
            wr = wr_v[...].astype(jnp.float32)
            gw = gw_v[...].astype(jnp.float32)
            r = jnp.zeros((8, 128), jnp.float32)
            gs = jnp.zeros((8, 128), jnp.float32)
            for j in range(D // 128):
                xj = xf[:, j * 128:(j + 1) * 128]
                r = r + xj * wr[j:j + 1, :]
                gs = gs + xj * gw[j:j + 1, :]
            r = jnp.sum(r, axis=-1, keepdims=True)
            gg = jax.nn.sigmoid(jnp.sum(gs, axis=-1, keepdims=True))
            bb = xf + (xf * 0.0 + y * jax.nn.sigmoid(r))
            b_scr[0] = (1.0 - gg) * bb
            b_scr[1] = jnp.broadcast_to(gg, (8, D))

        return carry

    jax.lax.fori_loop(0, H, body, 0)
    out = b_scr[1] * a_scr[...] + b_scr[0]
    o_ref[...] = out[0:B].astype(o_ref.dtype)


@jax.jit
def pallas_gated_mix__mha_block_cached__moe_arch_mod__decode_kernel(
    A_x: jax.Array,
    A_k_cache: jax.Array,
    A_v_cache: jax.Array,
    A_wq: jax.Array,
    A_wo: jax.Array,
    B_x: jax.Array,
    B_w_r: jax.Array,
    B_w_gate: jax.Array,
    B_w_up: jax.Array,
    B_w_down: jax.Array,
    gate_w: jax.Array,
):
    del B_x
    hbm = pl.BlockSpec(memory_space=pltpu.HBM)
    out = pl.pallas_call(
        _kernel,
        in_specs=[hbm] * 10,
        out_specs=pl.BlockSpec(memory_space=pltpu.VMEM),
        out_shape=jax.ShapeDtypeStruct((B, D), jnp.bfloat16),
        scratch_shapes=[
            pltpu.VMEM((B, D), jnp.bfloat16),
            pltpu.VMEM((D // 128, 128), jnp.bfloat16),
            pltpu.VMEM((D // 128, 128), jnp.bfloat16),
            pltpu.VMEM((D, H * DH), jnp.bfloat16),
            pltpu.VMEM((H * DH, D), jnp.bfloat16),
            pltpu.VMEM((D, F), jnp.bfloat16),
            pltpu.VMEM((D, F), jnp.bfloat16),
            pltpu.VMEM((F, D), jnp.bfloat16),
            pltpu.VMEM((NSLOT, B, CH, DH), jnp.bfloat16),
            pltpu.VMEM((NSLOT, B, CH, DH), jnp.bfloat16),
            pltpu.VMEM((H, 8, DH), jnp.float32),
            pltpu.VMEM((8, D), jnp.float32),
            pltpu.VMEM((8, F), jnp.float32),
            pltpu.VMEM((2, 8, D), jnp.float32),
            pltpu.SemaphoreType.DMA((NSLOT,)),
            pltpu.SemaphoreType.DMA((NSLOT,)),
            pltpu.SemaphoreType.DMA((8,)),
        ],
        compiler_params=pltpu.CompilerParams(
            vmem_limit_bytes=64 * 1024 * 1024,
            disable_bounds_checks=True,
        ),
    )(A_x.reshape(B, D), B_w_r.reshape(D // 128, 128), gate_w.reshape(D // 128, 128),
      A_k_cache, A_v_cache, A_wq, A_wo, B_w_gate, B_w_up, B_w_down)
    return out.reshape(B, 1, D)
```
